```python
import jax
import jax.numpy as jnp

def _softmax(x, axis=-1):
    return jax.nn.softmax(x, axis=axis)
def _gelu(x):
    return jax.nn.gelu(x, approximate=True)
def _silu(x):
    return jax.nn.silu(x)
def _sigmoid(x):
    return jax.nn.sigmoid(x)
def _layernorm(x, axis=-1, eps=1e-5):
    m = jnp.mean(x, axis=axis, keepdims=True)
    v = jnp.var(x, axis=axis, keepdims=True)
    return (x - m) / jnp.sqrt(v + eps)
def _scatter_add(tgt, idx, src, axis=0):
    return tgt.at[idx].add(src)
def _segment_sum(src, seg, n):
    return jax.ops.segment_sum(src, seg, n)
class _Rng:
    def __init__(self, key):
        self._k = key
    def _next(self):
        self._k, sub = jax.random.split(self._k)
        return sub
    def normal(self, shape):
        return jax.random.normal(self._next(), shape, dtype=jnp.bfloat16)
    def randint(self, lo, hi, shape):
        return jax.random.randint(self._next(), shape, lo, hi, dtype=jnp.int32)
    def uniform(self, shape, lo=0.0, hi=1.0):
        return jax.random.uniform(self._next(), shape, jnp.bfloat16, lo, hi)
    def permutation(self, n):
        return jax.random.permutation(self._next(), n)


kernel_name = 'interleave_layers__sliding_local_dilated__mixer_token_mlp__prompt'

def setup_inputs():
    _rng = _Rng(jax.random.key(int.from_bytes(__import__("os").urandom(4), "little")))
    _w = (lambda a: (lambda t: t.astype(jnp.bfloat16) if jnp.issubdtype(t.dtype, jnp.floating) else t)(jnp.asarray(a)))
    def _A_setup():
        B, S, D = 1, 2048, 1024
        return {
            "x": _w((lambda *s: _rng.normal(s) * 0.05)(B, S, D)),
            "wqkv": _w((lambda *s: _rng.normal(s) * 0.05)(D, 3 * D)),
            "wo": _w((lambda *s: _rng.normal(s) * 0.05)(D, D)),
        }
    _A_in = _A_setup()

    def _B_setup():
        B, S, D, F = 1, 2048, 1024, 3584
        return {
            "x": _w((lambda *s: _rng.normal(s) * 0.05)(B, S, D)),
            "w1": _w((lambda *s: _rng.normal(s) * 0.05)(S, F) * (S ** -0.5)),
            "b1": _w((lambda *s: _rng.normal(s) * 0.05)(F) * 0.02),
            "w2": _w((lambda *s: _rng.normal(s) * 0.05)(F, S) * (F ** -0.5)),
            "b2": _w((lambda *s: _rng.normal(s) * 0.05)(S) * 0.02),
        }
    _B_in = _B_setup()

    return {
        "A_x": _A_in["x"],
        "A_wqkv": _A_in["wqkv"],
        "A_wo": _A_in["wo"],
        "B_x": _B_in["x"],
        "B_w1": _B_in["w1"],
        "B_b1": _B_in["b1"],
        "B_w2": _B_in["w2"],
        "B_b2": _B_in["b2"],
    }

def reference(A_x, A_wqkv, A_wo, B_x, B_w1, B_b1, B_w2, B_b2):
    def _A_ref(x, wqkv, wo):
        B, S, D = x.shape
        H = 32; Dh = D // H
        W, dil = 8, 2
        qkv = (lambda x, *d: x.transpose(*d))((x @ wqkv).reshape(B, S, 3, H, Dh), 2, 0, 3, 1, 4)
        q, k, v = qkv[0], qkv[1], qkv[2]
        scale = Dh ** -0.5
        pos = jnp.arange(S)
        off = jnp.arange(W) * dil
        idx = pos[:, None] - off[None, :]
        mask = idx >= 0
        idx_c = jnp.where(mask, idx, 0).reshape(-1)
        kg = k[:, :, idx_c, :].reshape(B, H, S, W, Dh)
        vg = v[:, :, idx_c, :].reshape(B, H, S, W, Dh)
        logits = jnp.einsum("bhsd,bhswd->bhsw", q, kg) * scale
        logits = jnp.where(mask[None, None, :, :], logits, -1e9)
        attn = _softmax(logits, axis=-1)
        o = jnp.einsum("bhsw,bhswd->bhsd", attn, vg)
        return (lambda x, *d: x.transpose(*d))(o, 0, 2, 1, 3).reshape(B, S, D) @ wo

    def _B_ref(x, w1, b1, w2, b2):
        B, S, D = x.shape
        h = _layernorm(x, axis=-1)
        u = jnp.einsum("bsd,sf->bdf", h, w1) + b1
        u = _gelu(u)
        y = jnp.einsum("bdf,fs->bds", u, w2) + b2
        return (lambda x, *d: x.transpose(*d))(y, 0, 2, 1)

    x = A_x
    x = x + _A_ref(_layernorm(x, axis=-1), A_wqkv, A_wo)
    x = x + _B_ref(_layernorm(x, axis=-1), B_w1, B_b1, B_w2, B_b2)
    x = x + _A_ref(_layernorm(x, axis=-1), A_wqkv, A_wo)
    x = x + _B_ref(_layernorm(x, axis=-1), B_w1, B_b1, B_w2, B_b2)
    return x
```

```python
import jax
import jax.numpy as jnp
from jax import lax
import jax.experimental.pallas as pl
import jax.experimental.pallas.tpu as pltpu

S, D, F = 2048, 1024, 3584
H, DH, W, DIL = 32, 32, 8, 2
EPS = 1e-5
SB = 512
NS = S // SB
FC = 512
NF = F // FC
NG = 8
f32, bf16 = jnp.float32, jnp.bfloat16


def _ln_cols(x):
    m = jnp.mean(x, axis=0, keepdims=True)
    c = x - m
    v = jnp.mean(c * c, axis=0, keepdims=True)
    return c * lax.rsqrt(v + EPS)


def _gelu(x):
    z = 0.7978845608028654 * (x + 0.044715 * (x * x * x))
    return 0.5 * x * (1.0 + jnp.tanh(z))


def _sublane_sums(parts):
    row = lax.broadcasted_iota(jnp.int32, (8, 128), 0)
    for sh in (4, 2, 1):
        n = len(parts) // 2
        keep = (row & sh) == 0
        nxt = []
        for i in range(n):
            a, b = parts[i], parts[i + n]
            if sh == 4:
                nxt.append(jnp.where(keep, a, b) + pltpu.roll(jnp.where(keep, b, a), 4, 0))
            else:
                nxt.append(jnp.where(keep, a + pltpu.roll(a, 8 - sh, 0), b + pltpu.roll(b, sh, 0)))
        parts = nxt
    return parts[0]


def _attn_head(q_ref, k_ref, v_ref, o_ref, r0):
    rows = pl.ds(r0, DH)
    lane16 = lax.broadcasted_iota(jnp.int32, (DH, 128), 1)
    lane8 = lax.broadcasted_iota(jnp.int32, (8, 128), 1)
    row8 = lax.broadcasted_iota(jnp.int32, (8, 128), 0)
    kprev = vprev = None
    for t in range(S // 128):
        ls = pl.ds(t * 128, 128)
        q = q_ref[rows, ls]
        k = k_ref[rows, ls]
        v = v_ref[rows, ls]
        kr = [k] + [pltpu.roll(k, DIL * w, 1) for w in range(1, W)]
        vr = [v] + [pltpu.roll(v, DIL * w, 1) for w in range(1, W)]
        parts = []
        for w in range(W):
            kw = kr[w]
            if w > 0 and t > 0:
                kw = jnp.where(lane16 < DIL * w, kprev[w], kw)
            p = q * kw.astype(f32)
            parts.append((p[0:8] + p[8:16]) + (p[16:24] + p[24:32]))
        lg = _sublane_sums(parts) * (DH ** -0.5)
        if t == 0:
            lg = jnp.where(lane8 >= DIL * row8, lg, -1e9)
        m = jnp.max(lg, axis=0, keepdims=True)
        e = jnp.exp(lg - m)
        p = e * (1.0 / jnp.sum(e, axis=0, keepdims=True))
        acc = None
        if t == 0:
            v0 = jnp.broadcast_to(v.astype(f32)[:, 0:1], (DH, 128))
        for w in range(W):
            vw = vr[w]
            if w > 0 and t > 0:
                vw = jnp.where(lane16 < DIL * w, vprev[w], vw)
            vw = vw.astype(f32)
            if w > 0 and t == 0:
                vw = jnp.where(lane16 < DIL * w, v0, vw)
            term = jnp.broadcast_to(p[w:w + 1], (DH, 128)) * vw
            acc = term if acc is None else acc + term
        o_ref[rows, ls] = acc.astype(bf16)
        kprev, vprev = kr, vr


def _kernel(x_hbm, wqkv_hbm, wo_hbm, w1_hbm, b1_ref, w2_hbm, b2_ref, out_hbm,
            io_ref, wqkv_raw, wo_raw, wqkvT, woT, w1_ref, w2_ref,
            xT, hT, g_ref, oT, q_ref, k_ref, v_ref, sem_x, sem_q, sem_o, sem_1, sem_2, sem_out):

    def cp_x(i):
        return pltpu.make_async_copy(x_hbm.at[pl.ds(i * SB, SB)], io_ref.at[pl.ds(i * SB, SB)], sem_x.at[i])

    def cp_q(i):
        return pltpu.make_async_copy(wqkv_hbm.at[:, pl.ds(i * D, D)], wqkv_raw.at[i], sem_q.at[i])

    cp_o = pltpu.make_async_copy(wo_hbm, wo_raw, sem_o.at[0])

    def cp_1(i):
        return pltpu.make_async_copy(w1_hbm.at[:, pl.ds(i * FC, FC)], w1_ref.at[i], sem_1.at[i])

    def cp_2(i):
        return pltpu.make_async_copy(w2_hbm.at[:, pl.ds(i * SB, SB)], w2_ref.at[i], sem_2.at[i])

    def cp_out(i):
        return pltpu.make_async_copy(io_ref.at[pl.ds(i * SB, SB)], out_hbm.at[pl.ds(i * SB, SB)], sem_out.at[i])

    for i in range(NS):
        cp_x(i).start()
    for i in range(3):
        cp_q(i).start()
    cp_o.start()
    for i in range(NF):
        cp_1(i).start()
    for i in range(NS):
        cp_2(i).start()

    def lanes(i):
        return pl.ds(pl.multiple_of(i * SB, SB), SB)

    for i in range(NS):
        cp_x(i).wait()
        xt = io_ref[pl.ds(i * SB, SB), :].T.astype(f32)
        xT[:, pl.ds(i * SB, SB)] = xt
        hT[:, pl.ds(i * SB, SB)] = _ln_cols(xt).astype(bf16)

    for part in range(3):
        cp_q(part).wait()
        for j in range(NG):
            wqkvT[j, pl.ds(part * 128, 128), :] = wqkv_raw[part, :, pl.ds(j * 128, 128)].T

    def qkv(j, slot):
        r = jnp.dot(wqkvT[j], hT[...], preferred_element_type=f32)
        q_ref[slot] = r[0:128]
        k_ref[slot] = r[128:256].astype(bf16)
        v_ref[slot] = r[256:384].astype(bf16)

    def attn(j, slot):
        for h in range(4):
            _attn_head(q_ref.at[slot], k_ref.at[slot], v_ref.at[slot], oT.at[j], h * DH)

    def layer_a(first):
        qkv(0, 0)

        def body(jj, c):
            j = jj * 2
            qkv(j + 1, 1)
            attn(j, 0)
            qkv(j + 2, 0)
            attn(j + 1, 1)
            return c

        lax.fori_loop(0, NG // 2 - 1, body, 0)
        qkv(NG - 1, 1)
        attn(NG - 2, 0)
        if first:
            cp_o.wait()
            for j in range(NG):
                woT[pl.ds(j * 128, 128), :] = wo_raw[:, pl.ds(j * 128, 128)].T
        attn(NG - 1, 1)

        def proj(i, c):
            ob = oT[:, :, lanes(i)].reshape(D, SB)
            x = xT[:, lanes(i)] + jnp.dot(woT[...], ob, preferred_element_type=f32)
            xT[:, lanes(i)] = x
            hT[:, lanes(i)] = _ln_cols(_ln_cols(x)).astype(bf16)
            return c

        lax.fori_loop(0, NS, proj, 0)

    def mlp_up(first):
        def body(c, carry):
            u = jnp.dot(hT[...], w1_ref[c], preferred_element_type=f32) + b1_ref[c].astype(f32)
            g_ref[:, pl.ds(pl.multiple_of(c * FC, FC), FC)] = _gelu(u).astype(bf16)
            return carry

        if first:
            for c in range(NF):
                cp_1(c).wait()
        lax.fori_loop(0, NF, body, 0)

    def mlp_down(i):
        y = jnp.dot(g_ref[...], w2_ref[i], preferred_element_type=f32) + b2_ref[i].astype(f32)
        return xT[:, lanes(i)] + y

    layer_a(True)
    mlp_up(True)
    for i in range(NS):
        cp_2(i).wait()

    def down1(i, c):
        x = mlp_down(i)
        xT[:, lanes(i)] = x
        hT[:, lanes(i)] = _ln_cols(x).astype(bf16)
        return c

    lax.fori_loop(0, NS, down1, 0)
    layer_a(False)
    mlp_up(False)

    def down2(i, c):
        x = mlp_down(i)
        r = pl.multiple_of(i * SB, SB)
        io_ref[pl.ds(r, SB), :] = x.astype(bf16).T
        pltpu.make_async_copy(io_ref.at[pl.ds(r, SB)], out_hbm.at[pl.ds(r, SB)], sem_out.at[i]).start()
        return c

    lax.fori_loop(0, NS, down2, 0)
    for i in range(NS):
        cp_out(i).wait()


@jax.jit
def pallas_interleave_layers__sliding_local_dilated__mixer_token_mlp__prompt_kernel(
    A_x: jax.Array,
    A_wqkv: jax.Array,
    A_wo: jax.Array,
    B_x: jax.Array,
    B_w1: jax.Array,
    B_b1: jax.Array,
    B_w2: jax.Array,
    B_b2: jax.Array,
):
    del B_x
    hbm = pl.BlockSpec(memory_space=pl.ANY)
    vmem = pl.BlockSpec(memory_space=pltpu.VMEM)
    out = pl.pallas_call(
        _kernel,
        in_specs=[hbm, hbm, hbm, hbm, vmem, hbm, vmem],
        out_specs=hbm,
        out_shape=jax.ShapeDtypeStruct((S, D), bf16),
        scratch_shapes=[
            pltpu.VMEM((S, D), bf16),
            pltpu.VMEM((3, D, D), bf16),
            pltpu.VMEM((D, D), bf16),
            pltpu.VMEM((NG, 384, D), bf16),
            pltpu.VMEM((D, D), bf16),
            pltpu.VMEM((NF, S, FC), bf16),
            pltpu.VMEM((NS, F, SB), bf16),
            pltpu.VMEM((D, S), f32),
            pltpu.VMEM((D, S), bf16),
            pltpu.VMEM((D, F), bf16),
            pltpu.VMEM((NG, 128, S), bf16),
            pltpu.VMEM((2, 128, S), f32),
            pltpu.VMEM((2, 128, S), bf16),
            pltpu.VMEM((2, 128, S), bf16),
            pltpu.SemaphoreType.DMA((NS,)),
            pltpu.SemaphoreType.DMA((3,)),
            pltpu.SemaphoreType.DMA((1,)),
            pltpu.SemaphoreType.DMA((NF,)),
            pltpu.SemaphoreType.DMA((NS,)),
            pltpu.SemaphoreType.DMA((NS,)),
        ],
        compiler_params=pltpu.CompilerParams(vmem_limit_bytes=110 * 1024 * 1024),
    )(A_x.reshape(S, D), A_wqkv, A_wo, B_w1, B_b1.reshape(NF, 1, FC), B_w2, B_b2.reshape(NS, 1, SB))
    return out.reshape(1, S, D)
```

```python
import jax
import jax.numpy as jnp
from jax import lax
import jax.experimental.pallas as pl
import jax.experimental.pallas.tpu as pltpu

S, D, F = 2048, 1024, 3584
H, DH, W, DIL = 32, 32, 8, 2
EPS = 1e-5
SB = 512
NS = S // SB
FC = 512
NF = F // FC
NG = 8
f32, bf16 = jnp.float32, jnp.bfloat16


def _ln_cols(x):
    m = jnp.mean(x, axis=0, keepdims=True)
    c = x - m
    v = jnp.mean(c * c, axis=0, keepdims=True)
    return c * lax.rsqrt(v + EPS)


def _ln2_cols(x):
    m = jnp.mean(x, axis=0, keepdims=True)
    c = x - m
    v = jnp.mean(c * c, axis=0, keepdims=True)
    r = lax.rsqrt(v + EPS)
    return c * (r * lax.rsqrt(v * r * r + EPS))


def _gelu(x):
    z = 0.7978845608028654 * (x + 0.044715 * (x * x * x))
    return 0.5 * x * (1.0 + jnp.tanh(z))


def _sublane_sums(parts):
    row = lax.broadcasted_iota(jnp.int32, (8, 128), 0)
    for sh in (4, 2, 1):
        n = len(parts) // 2
        keep = (row & sh) == 0
        nxt = []
        for i in range(n):
            a, b = parts[i], parts[i + n]
            if sh == 4:
                nxt.append(jnp.where(keep, a, b) + pltpu.roll(jnp.where(keep, b, a), 4, 0))
            else:
                nxt.append(jnp.where(keep, a + pltpu.roll(a, 8 - sh, 0), b + pltpu.roll(b, sh, 0)))
        parts = nxt
    return parts[0]


def _attn_head(q_ref, k_ref, v_ref, o_ref, r0):
    rows = pl.ds(r0, DH)
    lane16 = lax.broadcasted_iota(jnp.int32, (DH, 128), 1)
    lane8 = lax.broadcasted_iota(jnp.int32, (8, 128), 1)
    row8 = lax.broadcasted_iota(jnp.int32, (8, 128), 0)
    kprev = vprev = None
    for t in range(S // 128):
        ls = pl.ds(t * 128, 128)
        q = q_ref[rows, ls]
        k = k_ref[rows, ls]
        v = v_ref[rows, ls]
        kr = [k] + [pltpu.roll(k, DIL * w, 1) for w in range(1, W)]
        vr = [v] + [pltpu.roll(v, DIL * w, 1) for w in range(1, W)]
        parts = []
        for w in range(W):
            kw = kr[w]
            if w > 0 and t > 0:
                kw = jnp.where(lane16 < DIL * w, kprev[w], kw)
            p = q * kw.astype(f32)
            parts.append((p[0:8] + p[8:16]) + (p[16:24] + p[24:32]))
        lg = _sublane_sums(parts) * (DH ** -0.5)
        if t == 0:
            lg = jnp.where(lane8 >= DIL * row8, lg, -1e9)
        m = jnp.max(lg, axis=0, keepdims=True)
        e = jnp.exp(lg - m)
        p = e * (1.0 / jnp.sum(e, axis=0, keepdims=True))
        acc = None
        if t == 0:
            v0 = jnp.broadcast_to(v.astype(f32)[:, 0:1], (DH, 128))
        for w in range(W):
            vw = vr[w]
            if w > 0 and t > 0:
                vw = jnp.where(lane16 < DIL * w, vprev[w], vw)
            vw = vw.astype(f32)
            if w > 0 and t == 0:
                vw = jnp.where(lane16 < DIL * w, v0, vw)
            term = jnp.broadcast_to(p[w:w + 1], (DH, 128)) * vw
            acc = term if acc is None else acc + term
        o_ref[rows, ls] = acc.astype(bf16)
        kprev, vprev = kr, vr


def _kernel(x_hbm, wqkv_hbm, wo_hbm, w1_hbm, b1_ref, w2_hbm, b2_ref, out_hbm,
            io_ref, wqkv_raw, wo_raw, wqkvT, woT, w1_ref, w2_ref,
            xT, hT, g_ref, oT, q_ref, k_ref, v_ref, sem_x, sem_q, sem_o, sem_1, sem_2, sem_out):

    def cp_x(i):
        return pltpu.make_async_copy(x_hbm.at[pl.ds(i * SB, SB)], io_ref.at[pl.ds(i * SB, SB)], sem_x.at[i])

    def cp_q(j, part):
        return pltpu.make_async_copy(wqkv_hbm.at[:, pl.ds(part * D + j * 128, 128)],
                                     wqkv_raw.at[j, part], sem_q.at[j * 3 + part])

    cp_o = pltpu.make_async_copy(wo_hbm, wo_raw, sem_o.at[0])

    def cp_1(i):
        return pltpu.make_async_copy(w1_hbm.at[:, pl.ds(i * FC, FC)], w1_ref.at[i], sem_1.at[i])

    def cp_2(i):
        return pltpu.make_async_copy(w2_hbm.at[:, pl.ds(i * SB, SB)], w2_ref.at[i], sem_2.at[i])

    def cp_out(i):
        return pltpu.make_async_copy(io_ref.at[pl.ds(i * SB, SB)], out_hbm.at[pl.ds(i * SB, SB)], sem_out.at[i])

    cp_x(0).start()

    def lanes(i):
        return pl.ds(pl.multiple_of(i * SB, SB), SB)

    for i in range(NS):
        cp_x(i).wait()
        if i == 0:
            for n in range(1, NS):
                cp_x(n).start()
            for part in range(3):
                cp_q(0, part).start()
        if i == NS - 1:
            for j in range(1, NG):
                for part in range(3):
                    cp_q(j, part).start()
            cp_o.start()
        xt = io_ref[pl.ds(i * SB, SB), :].T.astype(f32)
        xT[:, pl.ds(i * SB, SB)] = xt
        hT[:, pl.ds(i * SB, SB)] = _ln_cols(xt).astype(bf16)

    def qkv(j, slot):
        r = jnp.dot(wqkvT[j], hT[...], preferred_element_type=f32)
        q_ref[slot] = r[0:128]
        k_ref[slot] = r[128:256].astype(bf16)
        v_ref[slot] = r[256:384].astype(bf16)

    def attn(j, slot):
        for h in range(4):
            _attn_head(q_ref.at[slot], k_ref.at[slot], v_ref.at[slot], oT.at[j], h * DH)

    def proj():
        for i in range(NS):
            ls = pl.ds(i * SB, SB)
            x = xT[:, ls] + jnp.dot(woT[...], oT[:, :, ls].reshape(D, SB), preferred_element_type=f32)
            xT[:, ls] = x
            hT[:, ls] = _ln2_cols(x).astype(bf16)

    def layer_a(first):
        if first:
            for part in range(3):
                cp_q(0, part).wait()
                wqkvT[0, pl.ds(part * 128, 128)] = wqkv_raw[0, part].T
        qkv(0, 0)
        if first:
            for j in range(1, NG):
                for part in range(3):
                    cp_q(j, part).wait()
            cp_o.wait()
            for i in range(NF):
                cp_1(i).start()
            for i in range(NS):
                cp_2(i).start()
            for j in range(1, NG):
                for part in range(3):
                    wqkvT[j, pl.ds(part * 128, 128)] = wqkv_raw[j, part].T
            for j in range(NG):
                woT[:, pl.ds(j * 128, 128)] = wo_raw[j].T
        qkv(1, 1)
        attn(0, 0)

        def body(jj, c):
            j = jj * 2
            qkv(j + 2, 0)
            attn(j + 1, 1)
            qkv(j + 3, 1)
            attn(j + 2, 0)
            return c

        lax.fori_loop(0, NG // 2 - 1, body, 0)
        attn(NG - 1, 1)
        proj()

    def mlp_up(first):
        def body(c, carry):
            u = jnp.dot(hT[...], w1_ref[c], preferred_element_type=f32) + b1_ref[pl.ds(pl.multiple_of(c * FC, FC), FC)].astype(f32).reshape(1, FC)
            g_ref[:, pl.ds(pl.multiple_of(c * FC, FC), FC)] = _gelu(u).astype(bf16)
            return carry

        if first:
            for c in range(NF):
                cp_1(c).wait()
        lax.fori_loop(0, NF, body, 0)

    def mlp_down(i):
        y = jnp.dot(g_ref[...], w2_ref[i], preferred_element_type=f32) + b2_ref[lanes(i)].astype(f32).reshape(1, SB)
        return xT[:, lanes(i)] + y

    layer_a(True)
    mlp_up(True)
    for i in range(NS):
        cp_2(i).wait()

    def down1(i, c):
        x = mlp_down(i)
        xT[:, lanes(i)] = x
        hT[:, lanes(i)] = _ln_cols(x).astype(bf16)
        return c

    lax.fori_loop(0, NS, down1, 0)
    layer_a(False)
    mlp_up(False)

    def down2(i, c):
        x = mlp_down(i)
        r = pl.multiple_of(i * SB, SB)
        io_ref[pl.ds(r, SB), :] = x.astype(bf16).T
        pltpu.make_async_copy(io_ref.at[pl.ds(r, SB)], out_hbm.at[pl.ds(r, SB)], sem_out.at[i]).start()
        return c

    lax.fori_loop(0, NS, down2, 0)
    for i in range(NS):
        cp_out(i).wait()


@jax.jit
def pallas_interleave_layers__sliding_local_dilated__mixer_token_mlp__prompt_kernel(
    A_x: jax.Array,
    A_wqkv: jax.Array,
    A_wo: jax.Array,
    B_x: jax.Array,
    B_w1: jax.Array,
    B_b1: jax.Array,
    B_w2: jax.Array,
    B_b2: jax.Array,
):
    del B_x
    hbm = pl.BlockSpec(memory_space=pl.ANY)
    vmem = pl.BlockSpec(memory_space=pltpu.VMEM)
    out = pl.pallas_call(
        _kernel,
        in_specs=[hbm, hbm, hbm, hbm, vmem, hbm, vmem],
        out_specs=hbm,
        out_shape=jax.ShapeDtypeStruct((S, D), bf16),
        scratch_shapes=[
            pltpu.VMEM((S, D), bf16),
            pltpu.VMEM((NG, 3, D, 128), bf16),
            pltpu.VMEM((NG, 128, D), bf16),
            pltpu.VMEM((NG, 384, D), bf16),
            pltpu.VMEM((D, D), bf16),
            pltpu.VMEM((NF, S, FC), bf16),
            pltpu.VMEM((NS, F, SB), bf16),
            pltpu.VMEM((D, S), f32),
            pltpu.VMEM((D, S), bf16),
            pltpu.VMEM((D, F), bf16),
            pltpu.VMEM((NG, 128, S), bf16),
            pltpu.VMEM((2, 128, S), f32),
            pltpu.VMEM((2, 128, S), bf16),
            pltpu.VMEM((2, 128, S), bf16),
            pltpu.SemaphoreType.DMA((NS,)),
            pltpu.SemaphoreType.DMA((NG * 3,)),
            pltpu.SemaphoreType.DMA((1,)),
            pltpu.SemaphoreType.DMA((NF,)),
            pltpu.SemaphoreType.DMA((NS,)),
            pltpu.SemaphoreType.DMA((NS,)),
        ],
        compiler_params=pltpu.CompilerParams(vmem_limit_bytes=110 * 1024 * 1024, flags={'XLA_TPU_FORCE_LP_LLO_SCHEDULER': True}),
    )(A_x.reshape(S, D), A_wqkv, A_wo.reshape(NG, 128, D), B_w1, B_b1, B_w2, B_b2)
    return out.reshape(1, S, D)
```
